```python
import os as _os
_os.environ.setdefault("JAX_PLATFORMS", "cpu")
import jax
import jax.numpy as jnp

def _softmax(x, axis=-1):
    return jax.nn.softmax(x, axis=axis)
def _gelu(x):
    return jax.nn.gelu(x, approximate=True)
def _silu(x):
    return jax.nn.silu(x)
def _sigmoid(x):
    return jax.nn.sigmoid(x)
def _layernorm(x, axis=-1, eps=1e-5):
    m = jnp.mean(x, axis=axis, keepdims=True)
    v = jnp.var(x, axis=axis, keepdims=True)
    return (x - m) / jnp.sqrt(v + eps)
def _scatter_add(tgt, idx, src, axis=0):
    return tgt.at[idx].add(src)
def _segment_sum(src, seg, n):
    return jax.ops.segment_sum(src, seg, n)
class _Rng:
    def __init__(self, key):
        self._k = key
    def _next(self):
        self._k, sub = jax.random.split(self._k)
        return sub
    def normal(self, shape):
        return jax.random.normal(self._next(), shape, dtype=jnp.bfloat16)
    def randint(self, lo, hi, shape):
        return jax.random.randint(self._next(), shape, lo, hi, dtype=jnp.int32)
    def uniform(self, shape, lo=0.0, hi=1.0):
        return jax.random.uniform(self._next(), shape, jnp.bfloat16, lo, hi)
    def permutation(self, n):
        return jax.random.permutation(self._next(), n)


kernel_name = 'interleave_layers__sliding_block_cached__mixer_channel_mlp__decode'

def setup_inputs():
    _rng = _Rng(jax.random.key(int.from_bytes(__import__("os").urandom(4), "little")))
    _w = (lambda a: (lambda t: t.astype(jnp.bfloat16) if jnp.issubdtype(t.dtype, jnp.floating) else t)(jnp.asarray(a)))
    def _A_setup():
        B, Sq, D = 8, 1, 1024
        Hq, Hkv, Sk, Dh = 32, 4, 4096, 128
        assert Hq % Hkv == 0, (Hq, Hkv)
        return {
            "x": _w((lambda *s: _rng.normal(s) * 0.05)(B, Sq, D)),
            "k_cache": _w((lambda *s: _rng.normal(s) * 1.6)(B, Hkv, Sk, Dh)),
            "v_cache": _w((lambda *s: _rng.normal(s) * 0.8)(B, Hkv, Sk, Dh)),
            "wq": _w((lambda *s: _rng.normal(s) * 1.6)(D, Hq * Dh) * (D ** -0.5)),
            "wo": _w((lambda *s: _rng.normal(s) * 0.8)(Hq * Dh, D) * ((Hq * Dh) ** -0.5)),
        }
    _A_in = _A_setup()

    def _B_setup():
        B, S, D, F = 8, 1, 1024, 3584
        return {
            "x": _w((lambda *s: _rng.normal(s) * 0.05)(B, S, D)),
            "w1": _w((lambda *s: _rng.normal(s) * 0.4)(D, F) * (D ** -0.5)),
            "b1": _w((lambda *s: _rng.normal(s) * 0.4)(F)),
            "w2": _w((lambda *s: _rng.normal(s) * 0.4)(F, D) * (F ** -0.5)),
            "b2": _w((lambda *s: _rng.normal(s) * 0.1)(D)),
        }
    _B_in = _B_setup()

    return {
        "A_x": _A_in["x"],
        "A_k_cache": _A_in["k_cache"],
        "A_v_cache": _A_in["v_cache"],
        "A_wq": _A_in["wq"],
        "A_wo": _A_in["wo"],
        "B_x": _B_in["x"],
        "B_w1": _B_in["w1"],
        "B_b1": _B_in["b1"],
        "B_w2": _B_in["w2"],
        "B_b2": _B_in["b2"],
    }

def reference(A_x, A_k_cache, A_v_cache, A_wq, A_wo, B_x, B_w1, B_b1, B_w2, B_b2):
    def _A_ref(x, k_cache, v_cache, wq, wo):
        B, Sq, D = x.shape
        Hq, Dh = 32, 128
        Hkv, Sk = k_cache.shape[1], k_cache.shape[2]
        W = min(4096, max(256, Sk // 4))
        rep = Hq // Hkv
        q = (lambda x, *d: x.transpose(*d))((x @ wq).reshape(B, Sq, Hq, Dh), 0, 2, 1, 3)
        k = jnp.repeat(k_cache[:, :, Sk - W:, :], rep, axis=1)
        v = jnp.repeat(v_cache[:, :, Sk - W:, :], rep, axis=1)
        scores = jnp.einsum("bhqd,bhkd->bhqk", q, k) * (Dh ** -0.5)
        p = _softmax(scores, axis=-1)
        o = jnp.einsum("bhqk,bhkd->bhqd", p, v)
        return (lambda x, *d: x.transpose(*d))(o, 0, 2, 1, 3).reshape(B, Sq, Hq * Dh) @ wo

    def _B_ref(x, w1, b1, w2, b2):
        y = _layernorm(x, axis=-1)
        h = _gelu(jnp.einsum("bsd,df->bsf", y, w1) + b1)
        return jnp.einsum("bsf,fd->bsd", h, w2) + b2

    x = A_x
    x = x + _A_ref(_layernorm(x, axis=-1), A_k_cache, A_v_cache, A_wq, A_wo)
    x = x + _B_ref(_layernorm(x, axis=-1), B_w1, B_b1, B_w2, B_b2)
    x = x + _A_ref(_layernorm(x, axis=-1), A_k_cache, A_v_cache, A_wq, A_wo)
    x = x + _B_ref(_layernorm(x, axis=-1), B_w1, B_b1, B_w2, B_b2)
    return x
```

```python
import functools
import numpy as np
import jax
import jax.numpy as jnp
import jax.experimental.pallas as pl
import jax.experimental.pallas.tpu as pltpu

F32 = jnp.float32
BF16 = jnp.bfloat16
EPS = 1e-5
NSEM = 4


def _ln(x):
    m = jnp.mean(x, axis=-1, keepdims=True)
    d = x - m
    v = jnp.mean(d * d, axis=-1, keepdims=True)
    return d * jax.lax.rsqrt(v + EPS)


def _gelu(x):
    c = np.float32(np.sqrt(2.0 / np.pi))
    return 0.5 * x * (1.0 + jnp.tanh(c * (x + 0.044715 * (x * x * x))))


def _dot(a, b):
    return jnp.dot(a, b, preferred_element_type=F32)


def _kernel(x_h, k_h, v_h, wq_h, wo_h, w1_h, b1_h, w2_h, b2_h, o_ref,
            x_v, b1_v, b2_v, k_v, v_v, wq_v, wo_v, w1_v, w2_v, q_s, o_s, b1_f, b2_f, sems, ssem):
    B, G, W, Dh = k_v.shape
    Sk = k_h.shape[2]
    R = wq_v.shape[1] // Dh // G
    D, F = w1_v.shape
    scale = np.float32(Dh ** -0.5)

    cps = []
    for i in range(8):
        cps.append((wq_h.at[:, pl.ds(i * 512, 512)], wq_v.at[:, pl.ds(i * 512, 512)]))
    for b in range(B):
        cps.append((k_h.at[b, :, pl.ds(Sk - W, W), :], k_v.at[b]))
        cps.append((v_h.at[b, :, pl.ds(Sk - W, W), :], v_v.at[b]))
    for i in range(8):
        cps.append((wo_h.at[pl.ds(i * 512, 512)], wo_v.at[pl.ds(i * 512, 512)]))
    for i in range(7):
        cps.append((w1_h.at[:, pl.ds(i * 512, 512)], w1_v.at[:, pl.ds(i * 512, 512)]))
    for i in range(7):
        cps.append((w2_h.at[pl.ds(i * 512, 512)], w2_v.at[pl.ds(i * 512, 512)]))
    dmas = [pltpu.make_async_copy(s, t, sems.at[i % NSEM]) for i, (s, t) in enumerate(cps)]
    small = [pltpu.make_async_copy(s, t, ssem) for s, t in ((x_h, x_v), (b1_h, b1_v), (b2_h, b2_v))]
    dmas[0].start()
    for c in small:
        c.start()
    for i in range(1, NSEM):
        dmas[i].start()
    state = [0]

    def nxt():
        i = state[0]
        dmas[i].wait()
        if i + NSEM < len(dmas):
            dmas[i + NSEM].start()
        state[0] = i + 1

    for c in small:
        c.wait()
    b1_f[...] = b1_v[...].astype(F32)
    b2_f[...] = b2_v[...].astype(F32)
    x = x_v[...].astype(F32)

    def attn(x, first):
        y = _ln(x).astype(BF16)
        for i in range(8):
            if first:
                nxt()
            q = _dot(y, wq_v[:, i * 512:(i + 1) * 512])
            for j in range(4):
                q_s[pl.ds((i * 4 + j) * B, B), :] = q[:, j * 128:(j + 1) * 128]
        for b in range(B):
            if first:
                nxt()
            ps = []
            for g in range(G):
                qb = q_s[pl.ds(g * R * B + b, R, stride=B), :].astype(BF16)
                s = jax.lax.dot_general(qb, k_v[b, g], (((1,), (1,)), ((), ())),
                                        preferred_element_type=F32) * scale
                m = jnp.max(s, axis=-1, keepdims=True)
                p = jnp.exp(s - m)
                l = jnp.sum(p, axis=-1, keepdims=True)
                ps.append((p.astype(BF16), l))
            if first:
                nxt()
            for g in range(G):
                p, l = ps[g]
                o = _dot(p, v_v[b, g]) / l
                o_s[pl.ds(g * R * B + b, R, stride=B), :] = o
        acc = x
        for i in range(8):
            if first:
                nxt()
            o = jnp.concatenate([o_s[pl.ds((i * 4 + j) * B, B), :] for j in range(4)], axis=1).astype(BF16)
            acc = acc + _dot(o, wo_v[i * 512:(i + 1) * 512, :])
        return acc

    def mlp(x, first):
        y = _ln(_ln(x)).astype(BF16)
        hs = []
        for i in range(7):
            if first:
                nxt()
            t = _dot(y, w1_v[:, i * 512:(i + 1) * 512])
            bias = jnp.concatenate([jnp.broadcast_to(b1_f[pl.ds(i * 4 + j, 1), :], (B, 128)) for j in range(4)], axis=1)
            hs.append(_gelu(t + bias).astype(BF16))
        bias = jnp.concatenate([jnp.broadcast_to(b2_f[pl.ds(j, 1), :], (B, 128)) for j in range(8)], axis=1)
        acc = x + bias
        for i in range(7):
            if first:
                nxt()
            acc = acc + _dot(hs[i], w2_v[i * 512:(i + 1) * 512, :])
        return acc

    x = attn(x, True)
    x = mlp(x, True)
    x = attn(x, False)
    x = mlp(x, False)
    o_ref[...] = x.astype(o_ref.dtype)


@jax.jit
def pallas_interleave_layers__sliding_block_cached__mixer_channel_mlp__decode_kernel(A_x, A_k_cache, A_v_cache, A_wq, A_wo, B_x, B_w1, B_b1, B_w2, B_b2):
    B, Sq, D = A_x.shape
    _, G, Sk, Dh = A_k_cache.shape
    W = min(4096, max(256, Sk // 4))
    F = B_w1.shape[1]
    HD = A_wq.shape[1]
    any_ = pl.BlockSpec(memory_space=pl.ANY)
    out = pl.pallas_call(
        _kernel,
        out_shape=jax.ShapeDtypeStruct((B, D), A_x.dtype),
        in_specs=[any_] * 9,
        scratch_shapes=[
            pltpu.VMEM((B, D), BF16), pltpu.VMEM((F // 128, 128), BF16), pltpu.VMEM((D // 128, 128), BF16),
            pltpu.VMEM((B, G, W, Dh), BF16), pltpu.VMEM((B, G, W, Dh), BF16),
            pltpu.VMEM((D, HD), BF16), pltpu.VMEM((HD, D), BF16),
            pltpu.VMEM((D, F), BF16), pltpu.VMEM((F, D), BF16),
            pltpu.VMEM((HD // Dh * B, Dh), F32), pltpu.VMEM((HD // Dh * B, Dh), F32),
            pltpu.VMEM((F // 128, 128), F32), pltpu.VMEM((D // 128, 128), F32),
            pltpu.SemaphoreType.DMA((NSEM,)), pltpu.SemaphoreType.DMA,
        ],
        compiler_params=pltpu.CompilerParams(vmem_limit_bytes=100 * 1024 * 1024),
        name="fused",
    )(A_x.reshape(B, D), A_k_cache, A_v_cache, A_wq, A_wo, B_w1, B_b1.reshape(F // 128, 128), B_w2,
      B_b2.reshape(D // 128, 128))
    return out.reshape(B, Sq, D)
```

```python
import functools

import numpy as np
import jax
import jax.numpy as jnp
import jax.experimental.pallas as pl
import jax.experimental.pallas.tpu as pltpu

F32 = jnp.float32
BF16 = jnp.bfloat16
EPS = 1e-5
LANES = 128
NUM_SEMS = 6
QUEUE_LAG = 80
SOFTMAX_LAG = 4


def _gelu(x):
    c = np.float32(np.sqrt(2.0 / np.pi))
    return 0.5 * x * (1.0 + jnp.tanh(c * (x + 0.044715 * (x * x * x))))


def _dot(a, b):
    return jnp.dot(a, b, preferred_element_type=F32)


def _ln_stats(x):
    m = jnp.mean(x, axis=-1, keepdims=True)
    d = x - m
    v = jnp.mean(d * d, axis=-1, keepdims=True)
    return m, d, jax.lax.rsqrt(v + EPS)


def _softmax_parts(s):
    p = jnp.exp(s - jnp.max(s, axis=-1, keepdims=True))
    return p, 1.0 / jnp.sum(p, axis=-1, keepdims=True)


def _ds(start, size, mult):
    if isinstance(start, int):
        return pl.ds(start, size)
    return pl.ds(pl.multiple_of(start, mult), size)


def _start_copies(copies, sem, burst):
    for n, (src, dst) in enumerate(copies):
        low = burst == 0 or (n // burst) % 2 == 0
        pltpu.make_async_copy(src, dst, sem).start(priority=1 if low else 0)


def _row_streams(src, dst, rows, src_cols, dst_col0, num_units, copy_shape, burst, num_streams=8):
    (r0, r1), (c0, c1), (cr, cc) = rows, src_cols, copy_shape
    stream = (r1 - r0) // num_streams
    unit = stream // num_units
    offsets = [(s * stream + r, c) for r in range(0, unit, cr) for c in range(0, c1 - c0, cc)
               for s in range(num_streams)]

    def start(u, sem):
        span = _ds(r0 + u * unit, (num_streams - 1) * stream + unit, 8)
        src_u, dst_u = src.at[span], dst.at[span]
        _start_copies([(src_u.at[pl.ds(r, cr), pl.ds(c0 + c, cc)], dst_u.at[pl.ds(r, cr), pl.ds(dst_col0 + c, cc)])
                       for r, c in offsets], sem, burst)

    return num_units, len(offsets) // 2 if burst else len(offsets), start


def _window_streams(src, dst):
    B, G, W, _ = dst.shape
    unit, cr = W // 2, 64

    def start(u, sem):
        bs, r0 = pl.ds((u // 2) * 2, 2), (u % 2) * unit
        src_u = src.at[bs, :, _ds(src.shape[2] - W + r0, unit, cr), :]
        dst_u = dst.at[bs, :, _ds(r0, unit, cr), :]
        _start_copies([(src_u.at[b, g, pl.ds(r, cr), :], dst_u.at[b, g, pl.ds(r, cr), :])
                       for r in range(0, unit, cr) for b in range(2) for g in range(G)], sem, 2)

    return B, G * unit // cr, start


def _kernel(x_h, k_h, v_h, wq_h, wo_h, w1_h, b1_h, w2_h, b2_h, o_ref,
            x_v, b1_v, b2_v, k_v, kt_v, v_v, wq_v, wo_v, w1_v, w2_v,
            y_s, wq_sum, q_s, p_s, pinv_s, o_s, x1_s, w1_sum, h_s, b1_s, b2_s, x2_s, q2_s,
            sems, small_sem):
    B, G, W, Dh = k_v.shape
    D, F = w1_v.shape
    HD = wq_v.shape[1]
    R = HD // Dh // G
    NB = D // LANES
    scale = np.float32(Dh ** -0.5)

    def head_rows(g, b):
        return pl.ds(g * R * B + b, R, stride=B)

    def set_lhs(y):
        y_s[...] = jnp.concatenate([y, jnp.ones((B, D), F32)], axis=0).astype(BF16)

    def h_cols(j0, j1):
        return jnp.concatenate([h_s[j] for j in range(j0, j1)], axis=1).astype(BF16)

    def q_proj(u):
        cs = _ds(u * 512, 512, LANES)
        q = _dot(y_s[...], wq_v[:, cs])
        wq_sum[:, cs] = q[B:]
        for j in range(4):
            q_s[_ds((u * 4 + j) * B, B, B), :] = q[:B, j * Dh:(j + 1) * Dh] * scale

    def scores(b):
        for g in range(G):
            kt = k_v[b, g].T
            kt_v[b, g] = kt
            p, pinv = _softmax_parts(_dot(q_s[head_rows(g, b), :].astype(BF16), kt))
            p_s[b, g] = p
            pinv_s[b, g] = jnp.broadcast_to(pinv, (R, Dh))

    def values(b):
        for g in range(G):
            o_s[head_rows(g, b), :] = _dot(p_s[b, g].astype(BF16), v_v[b, g]) * pinv_s[b, g]

    def out_proj(u):
        acc = x1_s[...]
        for c in range(2):
            o = jnp.concatenate([o_s[_ds((u * 4 + c * 2 + j) * B, B, B), :] for j in range(2)], axis=1)
            acc = acc + _dot(o.astype(BF16), wo_v[_ds(u * 512 + c * 256, 256, 256), :])
        x1_s[...] = acc

        @pl.when(u == HD // 512 - 1)
        def _():
            _, d1, r1 = _ln_stats(acc)
            _, d2, r2 = _ln_stats(d1 * r1)
            set_lhs(d2 * r2)

    def mlp_in(u):
        cs = _ds(u * 512, 512, LANES)
        t = _dot(y_s[...], w1_v[:, cs])
        w1_sum[:, cs] = t[B:]
        h = _gelu(t[:B] + b1_s[:, cs])
        for j in range(4):
            h_s[u * 4 + j] = h[:, j * LANES:(j + 1) * LANES]

    def mlp_out(j):
        cs = pl.ds(j * LANES, LANES)
        xb = (x1_s[:, cs] + _dot(h_cols(0, F // LANES), w2_v[j]) + b2_s[:, cs]).astype(BF16)
        x2_s[:, cs] = xb.astype(F32)
        for n in range(0, HD, 1024):
            q2_s[:, n:n + 1024] += _dot(xb, wq_v[cs, n:n + 1024])

    starts, works, num_low = [], [], []

    def add_group(streams, buf, num_work=0, work=None):
        num_units, low, start = streams
        sem = sems.at[len(starts) % NUM_SEMS]
        starts.append((len(num_low), num_units, lambda u: start(u, sem)))
        num_low.extend([low] * num_units)

        def wait():
            pltpu.make_async_copy(buf, buf, sem).wait()

        def wait_and_work(u):
            pl.when(u == 0)(wait)
            work(u)

        if num_work:
            works.append((len(num_low) - 1, num_work, wait_and_work))
        return wait

    add_group(_row_streams(wq_h, wq_v, (0, D), (0, HD), 0, 8, (8, 512), 4), wq_v, HD // 512, q_proj)
    add_group(_window_streams(k_h, k_v), k_v, B, scores)
    add_group(_window_streams(v_h, v_v), v_v, B, values)
    add_group(_row_streams(wo_h, wo_v, (0, HD), (0, D), 0, 8, (8, 1024), 2), wo_v, HD // 512, out_proj)
    add_group(_row_streams(w1_h, w1_v, (0, D), (0, 2048), 0, 8, (8, 1024), 2),
              w1_v.at[:, pl.ds(0, 2048)], 4, mlp_in)
    add_group(_row_streams(w1_h, w1_v, (0, D), (2048, F), 2048, 8, (8, 768), 2),
              w1_v.at[:, pl.ds(2048, F - 2048)], 3, lambda u: mlp_in(u + 4))
    for j in range(NB - 1):
        add_group(_row_streams(w2_h, w2_v.at[j], (0, F), (j * LANES, (j + 1) * LANES), 0, 2, (32, LANES), 4),
                  w2_v.at[j], 1, lambda u, j=j: mlp_out(j))
    last = []
    for r0, r1, cr, burst, ns in ((0, 2048, 32, 4, 8), (2048, 3072, 1024, 0, 1), (3072, F, F - 3072, 0, 1)):
        streams = _row_streams(w2_h, w2_v.at[NB - 1], (r0, r1), (D - LANES, D), 0, 1, (cr, LANES), burst, ns)
        last.append((r0, r1, add_group(streams, w2_v.at[NB - 1, pl.ds(r0, r1 - r0)])))

    num_steps = len(num_low)
    t_free = 0
    for i, (t, n, f) in enumerate(works):
        queued = 0
        while queued < QUEUE_LAG and t + 1 < num_steps:
            t += 1
            queued += num_low[t]
        t = min(max(t, t_free), num_steps - 1)
        works[i] = (t, n, f)
        t_free = t + n
        assert t_free <= num_steps
        assert i + NUM_SEMS >= len(starts) or t < starts[i + NUM_SEMS][0]

    small = [pltpu.make_async_copy(s, d, small_sem) for s, d in ((x_h, x_v), (b1_h, b1_v), (b2_h, b2_v))]
    for c in small:
        c.start()

    def setup():
        for c in small:
            c.wait()
        for src, dst in ((b1_v, b1_s), (b2_v, b2_s)):
            bias = src[...].astype(F32)
            for j in range(bias.shape[0]):
                dst[:, j * LANES:(j + 1) * LANES] = jnp.broadcast_to(bias[j:j + 1, :], (B, LANES))
        x = x_v[...].astype(F32)
        x1_s[...] = x
        _, d, r = _ln_stats(x)
        set_lhs(d * r)
        q2_s[...] = jnp.zeros(q2_s.shape, F32)

    def step(t, carry):
        for t0, n, f in starts + [(0, 1, lambda u: setup())] + works:
            pl.when(jnp.logical_and(t >= t0, t < t0 + n))(functools.partial(f, t - t0))
        return carry

    jax.lax.fori_loop(0, num_steps, step, 0)

    acc = x1_s[:, D - LANES:]
    for r0, r1, wait in last:
        h = h_cols(r0 // LANES, r1 // LANES)
        wait()
        acc = acc + _dot(h, w2_v[NB - 1, r0:r1, :])
    xb = (acc + b2_s[:, D - LANES:]).astype(BF16)

    x2 = jnp.concatenate([x2_s[...], xb.astype(F32)], axis=1)
    m, _, r = _ln_stats(x2)
    r = r * scale
    for g in range(G):
        cs = slice(g * R * Dh, (g + 1) * R * Dh)
        q = (q2_s[:, cs] + _dot(xb, wq_v[D - LANES:, cs]) - m * wq_sum[:, cs]) * r
        for j in range(R):
            q_s[pl.ds((g * R + j) * B, B), :] = q[:, j * Dh:(j + 1) * Dh]

    pairs = [(g, b) for g in range(G) for b in range(B)]
    probs = []
    for i in range(len(pairs) + SOFTMAX_LAG):
        if i < len(pairs):
            g, b = pairs[i]
            p, pinv = _softmax_parts(_dot(q_s[head_rows(g, b), :].astype(BF16), kt_v[b, g]))
            probs.append((p.astype(BF16), pinv))
        if i >= SOFTMAX_LAG:
            g, b = pairs[i - SOFTMAX_LAG]
            p, pinv = probs[i - SOFTMAX_LAG]
            o_s[head_rows(g, b), :] = _dot(p, v_v[b, g]) * pinv

    acc = x2
    for i in range(HD // 256):
        o = jnp.concatenate([o_s[pl.ds((i * 2 + j) * B, B), :] for j in range(2)], axis=1)
        acc = acc + _dot(o.astype(BF16), wo_v[i * 256:(i + 1) * 256, :])
    x3b = acc.astype(BF16)
    x3 = x3b.astype(F32)

    m1, d1, r1 = _ln_stats(x3)
    m2, _, r2 = _ln_stats(d1 * r1)
    gain = r1 * r2
    shift = m1 * gain + m2 * r2
    hs = []
    for i in range(F // 512):
        cs = slice(i * 512, (i + 1) * 512)
        t = _dot(x3b, w1_v[:, cs])
        hs.append(_gelu(t * gain - shift * w1_sum[:, cs] + b1_s[:, cs]).astype(BF16))
    acc = x3 + b2_s[...]
    for i in range(F // 512):
        w2 = jnp.concatenate([w2_v[j, i * 512:(i + 1) * 512, :] for j in range(NB)], axis=1)
        acc = acc + _dot(hs[i], w2)
    o_ref[...] = acc.astype(o_ref.dtype)


@jax.jit
def pallas_interleave_layers__sliding_block_cached__mixer_channel_mlp__decode_kernel(
    A_x: jax.Array,
    A_k_cache: jax.Array,
    A_v_cache: jax.Array,
    A_wq: jax.Array,
    A_wo: jax.Array,
    B_x: jax.Array,
    B_w1: jax.Array,
    B_b1: jax.Array,
    B_w2: jax.Array,
    B_b2: jax.Array,
):
    del B_x
    B, Sq, D = A_x.shape
    _, G, Sk, Dh = A_k_cache.shape
    W = min(4096, max(256, Sk // 4))
    F = B_w1.shape[1]
    HD = A_wq.shape[1]
    R = HD // Dh // G
    assert (B, Sq, D, G, W, Dh, HD, F) == (8, 1, 1024, 4, 1024, 128, 4096, 3584)

    out = pl.pallas_call(
        _kernel,
        out_shape=jax.ShapeDtypeStruct((B, D), A_x.dtype),
        in_specs=[pl.BlockSpec(memory_space=pl.ANY)] * 9,
        scratch_shapes=[
            pltpu.VMEM((B, D), BF16),
            pltpu.VMEM((F // LANES, LANES), BF16),
            pltpu.VMEM((D // LANES, LANES), BF16),
            pltpu.VMEM((B, G, W, Dh), BF16),
            pltpu.VMEM((B, G, Dh, W), BF16),
            pltpu.VMEM((B, G, W, Dh), BF16),
            pltpu.VMEM((D, HD), BF16),
            pltpu.VMEM((HD, D), BF16),
            pltpu.VMEM((D, F), BF16),
            pltpu.VMEM((D // LANES, F, LANES), BF16),
            pltpu.VMEM((2 * B, D), BF16),
            pltpu.VMEM((B, HD), F32),
            pltpu.VMEM((HD // Dh * B + 8, Dh), F32),
            pltpu.VMEM((B, G, R, W), F32),
            pltpu.VMEM((B, G, R, Dh), F32),
            pltpu.VMEM((HD // Dh * B + 8, Dh), F32),
            pltpu.VMEM((B, D), F32),
            pltpu.VMEM((B, F), F32),
            pltpu.VMEM((F // LANES, B, LANES), F32),
            pltpu.VMEM((B, F), F32),
            pltpu.VMEM((B, D), F32),
            pltpu.VMEM((B, D - LANES), F32),
            pltpu.VMEM((B, HD), F32),
            pltpu.SemaphoreType.DMA((NUM_SEMS,)),
            pltpu.SemaphoreType.DMA,
        ],
        compiler_params=pltpu.CompilerParams(
            vmem_limit_bytes=100 * 1024 * 1024,
            disable_bounds_checks=True,
            disable_semaphore_checks=True,
        ),
    )(A_x.reshape(B, D), A_k_cache, A_v_cache, A_wq, A_wo, B_w1, B_b1.reshape(F // LANES, LANES),
      B_w2, B_b2.reshape(D // LANES, LANES))
    return out.reshape(B, Sq, D)
```
